```python
import os as _os
_os.environ.setdefault("JAX_PLATFORMS", "cpu")
import jax
import jax.numpy as jnp

def _softmax(x, axis=-1):
    return jax.nn.softmax(x, axis=axis)
def _gelu(x):
    return jax.nn.gelu(x, approximate=True)
def _silu(x):
    return jax.nn.silu(x)
def _sigmoid(x):
    return jax.nn.sigmoid(x)
def _layernorm(x, axis=-1, eps=1e-5):
    m = jnp.mean(x, axis=axis, keepdims=True)
    v = jnp.var(x, axis=axis, keepdims=True)
    return (x - m) / jnp.sqrt(v + eps)
def _scatter_add(tgt, idx, src, axis=0):
    return tgt.at[idx].add(src)
def _segment_sum(src, seg, n):
    return jax.ops.segment_sum(src, seg, n)
class _Rng:
    def __init__(self, key):
        self._k = key
    def _next(self):
        self._k, sub = jax.random.split(self._k)
        return sub
    def normal(self, shape):
        return jax.random.normal(self._next(), shape, dtype=jnp.bfloat16)
    def randint(self, lo, hi, shape):
        return jax.random.randint(self._next(), shape, lo, hi, dtype=jnp.int32)
    def uniform(self, shape, lo=0.0, hi=1.0):
        return jax.random.uniform(self._next(), shape, jnp.bfloat16, lo, hi)
    def permutation(self, n):
        return jax.random.permutation(self._next(), n)


kernel_name = 'sequential_preLN__ssm_conv_h3__mixer_s_mlp__prompt'

def setup_inputs():
    _rng = _Rng(jax.random.key(int.from_bytes(__import__("os").urandom(4), "little")))
    _w = (lambda a: (lambda t: t.astype(jnp.bfloat16) if jnp.issubdtype(t.dtype, jnp.floating) else t)(jnp.asarray(a)))
    def _A_setup():
        B, S, D = 1, 2048, 640
        ks = 4
        return {
            "q": _w((lambda *s: _rng.normal(s) * 0.05)(B, S, D)),
            "k": _w((lambda *s: _rng.normal(s) * 0.05)(B, S, D)),
            "v": _w((lambda *s: _rng.normal(s) * 0.05)(B, S, D)),
            "shift_k": _w((lambda *s: _rng.normal(s) * 0.05)(D, ks) * 0.5),
            "ssm_k": _w((lambda *s: _rng.normal(s) * 0.05)(D, S) * (1.0 / S ** 0.5)),
            "ssm_D": _w((lambda *s: _rng.normal(s) * 0.05)(D)),
        }
    _A_in = _A_setup()

    def _B_setup():
        B, S, D, F = 1, 2048, 640, 1728
        return {
            "x":  _w((lambda *s: _rng.normal(s) * 0.05)(B, S, D)),
            "w1": _w((lambda *s: _rng.normal(s) * 0.8)(D, D) * (D ** -0.5)),
            "w2": _w((lambda *s: _rng.normal(s) * 0.8)(D, D) * (D ** -0.5)),
            "w3": _w((lambda *s: _rng.normal(s) * 0.8)(D, F) * (D ** -0.5)),
            "w4": _w((lambda *s: _rng.normal(s) * 0.8)(F, D) * (F ** -0.5)),
        }
    _B_in = _B_setup()

    return {
        "A_q": _A_in["q"],
        "A_k": _A_in["k"],
        "A_v": _A_in["v"],
        "A_shift_k": _A_in["shift_k"],
        "A_ssm_k": _A_in["ssm_k"],
        "A_ssm_D": _A_in["ssm_D"],
        "B_x": _B_in["x"],
        "B_w1": _B_in["w1"],
        "B_w2": _B_in["w2"],
        "B_w3": _B_in["w3"],
        "B_w4": _B_in["w4"],
    }

def reference(A_q, A_k, A_v, A_shift_k, A_ssm_k, A_ssm_D, B_x, B_w1, B_w2, B_w3, B_w4):
    def _A_ref(q, k, v, shift_k, ssm_k, ssm_D):
        B, S, D = q.shape
        ks = shift_k.shape[-1]
        k_pad = jnp.pad(k, ((0, 0), (ks - 1, 0), (0, 0)))
        k_shift = jnp.zeros_like(k)
        for t in range(ks):
            k_shift = k_shift + k_pad[:, t:t + S, :] * shift_k[:, ks - 1 - t][None, None, :]
        kv = k_shift * v
        L = 2 * S
        kv_pad = jnp.pad(kv, ((0, 0), (0, S), (0, 0)))
        kf_pad = jnp.pad(ssm_k, ((0, 0), (0, S)))
        kv_f = (lambda x, axes=(-2,-1): jnp.fft.rfft2(x.astype(jnp.float32), axes=axes))(kv_pad[:, None, :, :], axes=(1, 2))
        kf_f = (lambda x, axes=(-2,-1): jnp.fft.rfft2(x.astype(jnp.float32), axes=axes))(kf_pad[:, None, :], axes=(1, 2))
        kf_f = (lambda x, *d: x.transpose(*d))(kf_f, 1, 2, 0)
        y_f = kv_f * kf_f[None, :, :, :]
        y = (lambda x, s, axes=(-2,-1): jnp.fft.irfft2(x, s=s, axes=axes).astype(jnp.bfloat16))(y_f, (1, L), axes=(1, 2))[:, 0, :S, :]
        y = y + kv * ssm_D[None, None, :]
        return q * y

    def _B_ref(x, w1, w2, w3, w4):
        B, S, D = x.shape
        h = _gelu(_layernorm(x, axis=-1) @ w1)
        c = D // 4
        g0 = jnp.pad(h[:, :, 0*c:1*c], ((0, 0), (1, 0), (0, 0)))[:, :S, :]
        g1 = jnp.pad(h[:, :, 1*c:2*c], ((0, 0), (0, 1), (0, 0)))[:, 1:, :]
        g2 = jnp.pad(h[:, :, 2*c:3*c], ((0, 0), (2, 0), (0, 0)))[:, :S, :]
        g3 = jnp.pad(h[:, :, 3*c:   ], ((0, 0), (0, 2), (0, 0)))[:, 2:, :]
        hs = jnp.concatenate([g0, g1, g2, g3], axis=-1) @ w2
        x1 = x + hs
        h2 = _gelu(_layernorm(x1, axis=-1) @ w3) @ w4
        return x1 + h2

    x = A_q
    h = x + _A_ref(_layernorm(x, axis=-1), A_k, A_v, A_shift_k, A_ssm_k, A_ssm_D)
    h2 = h + _B_ref(_layernorm(h, axis=-1), B_w1, B_w2, B_w3, B_w4)
    return h2
```

```python
import numpy as np
import jax
import jax.numpy as jnp
from jax import lax
import jax.experimental.pallas as pl
import jax.experimental.pallas.tpu as pltpu

S, D, F, KS = 2048, 640, 1728, 4
N = 2 * S
R = 64
NK2 = 33
HP = 40
TM = 256
EPS = 1e-5


def _consts():
    n2 = np.arange(32)
    k2 = np.arange(NK2)
    ang = 2 * np.pi * np.outer(k2, n2) / R
    f1 = np.zeros((2 * HP, 32), np.float64)
    f1[:NK2] = np.cos(ang)
    f1[HP:HP + NK2] = -np.sin(ang)
    n1 = np.arange(R)
    k1 = np.arange(R)
    mf = np.zeros((NK2, 128, 128), np.float64)
    mi = np.zeros((NK2, 128, 128), np.float64)
    for q in range(NK2):
        a = 2 * np.pi * np.outer(R * k1 + q, n1) / N
        c, s = np.cos(a), np.sin(a)
        mf[q] = np.block([[c, s], [-s, c]])
        mi[q] = np.block([[c.T, -s.T], [s.T, c.T]])
    g = np.zeros((32, 2 * HP), np.float64)
    w = np.full(NK2, 2.0); w[0] = 1.0; w[32] = 1.0
    g[:, :NK2] = np.cos(ang).T * w / N
    g[:, HP:HP + NK2] = -np.sin(ang).T * w / N
    bf = jnp.bfloat16
    return (jnp.asarray(f1, bf), jnp.asarray(mf, bf), jnp.asarray(mi, bf),
            jnp.asarray(g, bf))


def _ln(x):
    m = jnp.mean(x, axis=-1, keepdims=True)
    xc = x - m
    v = jnp.mean(xc * xc, axis=-1, keepdims=True)
    return xc * lax.rsqrt(v + EPS)


def _dot(a, b):
    return jnp.dot(a, b, preferred_element_type=jnp.float32)


def _sld(ref, start, size, stride):
    return jnp.concatenate(
        [ref[j, pl.ds(start, size, stride=stride), :] for j in range(D // 128)], axis=1)


def _sst(ref, start, size, stride, val):
    for j in range(D // 128):
        ref[j, pl.ds(start, size, stride=stride), :] = val[:, j * 128:(j + 1) * 128]


def _ld(ref, r, size):
    return jnp.concatenate([ref[j, pl.ds(r, size), :] for j in range(D // 128)], axis=1)


def _st(ref, r, size, val):
    for j in range(D // 128):
        ref[j, pl.ds(r, size), :] = val[:, j * 128:(j + 1) * 128]


def _kernel(q_ref, k_ref, v_ref, sh_ref, kt_ref, dd_ref, w1_ref, w2_ref, w3_ref, w4_ref,
            f1_ref, mf_ref, mi_ref, g_ref, o_ref,
            kpad, kv_s, ra, rb, bo, y_s, h_s, h1_s):
    bf = jnp.bfloat16
    f32 = jnp.float32
    kpad[0:8, :] = jnp.zeros((8, D), f32)
    kpad[8:, :] = k_ref[...].astype(f32)

    def p1(i, c):
        r = pl.multiple_of(i * TM, TM)
        w = kpad[pl.ds(r, TM + 8), :]
        acc = w[8:] * sh_ref[0:1, :]
        for u in range(1, KS):
            acc = acc + w[8 - u:8 - u + TM] * sh_ref[u:u + 1, :]
        _st(kv_s, r, TM, acc * v_ref[pl.ds(r, TM), :].astype(f32))
        return c
    lax.fori_loop(0, S // TM, p1, 0)

    f1 = f1_ref[...]

    def s1(n1, c):
        xa = _sld(kv_s, n1, 32, R).astype(bf)
        xb = _sld(kt_ref, n1, 32, R).astype(bf)
        a = _dot(f1, xa)
        b = _dot(f1, xb)
        _sst(ra, n1, HP, 128, a[:HP])
        _sst(ra, n1 + 64, HP, 128, a[HP:])
        _sst(rb, n1, HP, 128, b[:HP])
        _sst(rb, n1 + 64, HP, 128, b[HP:])
        return c
    lax.fori_loop(0, R, s1, 0)

    def s2(q, c):
        r = pl.multiple_of(q * 128, 128)
        xa = _dot(mf_ref[q], _ld(ra, r, 128).astype(bf))
        xb = _dot(mf_ref[q], _ld(rb, r, 128).astype(bf))
        ar, ai, br, bi = xa[:64], xa[64:], xb[:64], xb[64:]
        yy = jnp.concatenate([ar * br - ai * bi, ar * bi + ai * br], axis=0)
        _st(bo, r, 128, _dot(mi_ref[q], yy.astype(bf)))
        return c
    lax.fori_loop(0, NK2, s2, 0)
    bo[:, NK2 * 128:, :] = jnp.zeros((D // 128, (HP - NK2) * 128, 128), f32)

    g = g_ref[...]

    def s3(n1, c):
        z = jnp.concatenate([_sld(bo, n1, HP, 128), _sld(bo, n1 + 64, HP, 128)], axis=0)
        _sst(y_s, n1, 32, R, _dot(g, z.astype(bf)))
        return c
    lax.fori_loop(0, R, s3, 0)

    h1_s[0:8, :] = jnp.zeros((8, D), f32)
    h1_s[S + 8:, :] = jnp.zeros((8, D), f32)

    def p3(i, c):
        r = pl.multiple_of(i * TM, TM)
        x = q_ref[pl.ds(r, TM), :].astype(f32)
        yy = _ld(y_s, r, TM) + _ld(kv_s, r, TM) * dd_ref[...]
        h = x + _ln(x) * yy
        h_s[pl.ds(r, TM), :] = h
        t = _ln(_ln(h))
        h1_s[pl.ds(r + 8, TM), :] = jax.nn.gelu(_dot(t.astype(bf), w1_ref[...]), approximate=True)
        return c
    lax.fori_loop(0, S // TM, p3, 0)

    col = lax.broadcasted_iota(jnp.int32, (TM, D), 1)
    c4 = D // 4

    def p4(i, c):
        r = pl.multiple_of(i * TM, TM)
        w = h1_s[pl.ds(r, TM + 16), :]
        hs_in = jnp.where(
            col < c4, w[7:7 + TM],
            jnp.where(col < 2 * c4, w[9:9 + TM],
                      jnp.where(col < 3 * c4, w[6:6 + TM], w[10:10 + TM])))
        h = h_s[pl.ds(r, TM), :]
        x1 = _ln(h) + _dot(hs_in.astype(bf), w2_ref[...])
        a = jax.nn.gelu(_dot(_ln(x1).astype(bf), w3_ref[...]), approximate=True)
        h2 = _dot(a.astype(bf), w4_ref[...])
        o_ref[pl.ds(r, TM), :] = (h + x1 + h2).astype(o_ref.dtype)
        return c
    lax.fori_loop(0, S // TM, p4, 0)


@jax.jit
def pallas_sequential_preLN__ssm_conv_h3__mixer_s_mlp__prompt_kernel(
    A_q, A_k, A_v, A_shift_k, A_ssm_k, A_ssm_D, B_x, B_w1, B_w2, B_w3, B_w4):
    f1, mf, mi, g = _consts()
    f32 = jnp.float32
    vm = lambda shape: pltpu.VMEM(shape, f32)
    out = pl.pallas_call(
        _kernel,
        out_shape=jax.ShapeDtypeStruct((S, D), A_q.dtype),
        scratch_shapes=[
            vm((S + 8, D)), vm((5, S, 128)), vm((5, HP * 128, 128)), vm((5, HP * 128, 128)),
            vm((5, HP * 128, 128)), vm((5, S, 128)), vm((S, D)), vm((S + 16, D)),
        ],
        compiler_params=pltpu.CompilerParams(vmem_limit_bytes=100 * 1024 * 1024),
    )(A_q.reshape(S, D), A_k.reshape(S, D), A_v.reshape(S, D),
      A_shift_k.T.astype(f32), A_ssm_k.reshape(5, 128, S).transpose(0, 2, 1).astype(f32), A_ssm_D.reshape(1, D).astype(f32),
      B_w1, B_w2, B_w3, B_w4, f1, mf, mi, g)
    return out.reshape(1, S, D)
```

```python
import numpy as np
import jax
import jax.numpy as jnp
from jax import lax
import jax.experimental.pallas as pl
import jax.experimental.pallas.tpu as pltpu

S, D, F, KS = 2048, 640, 1728, 4
N = 2 * S
R = 64
NK2 = 33
HP = 40
TM = 256
EPS = 1e-5


def _consts():
    n2 = np.arange(32)
    k2 = np.arange(NK2)
    ang = 2 * np.pi * np.outer(k2, n2) / R
    f1 = np.zeros((2 * HP, 32), np.float64)
    f1[:NK2] = np.cos(ang)
    f1[HP:HP + NK2] = -np.sin(ang)
    n1 = np.arange(R)
    k1 = np.arange(R)
    mf = np.zeros((NK2, 128, 128), np.float64)
    mi = np.zeros((NK2, 128, 128), np.float64)
    for q in range(NK2):
        a = 2 * np.pi * np.outer(R * k1 + q, n1) / N
        c, s = np.cos(a), np.sin(a)
        mf[q] = np.block([[c, s], [-s, c]])
        mi[q] = np.block([[c.T, -s.T], [s.T, c.T]])
    g = np.zeros((32, 2 * HP), np.float64)
    w = np.full(NK2, 2.0); w[0] = 1.0; w[32] = 1.0
    g[:, :NK2] = np.cos(ang).T * w / N
    g[:, HP:HP + NK2] = -np.sin(ang).T * w / N
    bf = jnp.bfloat16
    e8 = np.eye(8)
    return (jnp.asarray(np.kron(f1, e8), bf), jnp.asarray(mf, bf), jnp.asarray(mi, bf),
            jnp.asarray(np.kron(g, e8), bf))


def _ln(x):
    m = jnp.mean(x, axis=-1, keepdims=True)
    xc = x - m
    v = jnp.mean(xc * xc, axis=-1, keepdims=True)
    return xc * lax.rsqrt(v + EPS)


def _dot(a, b):
    return jnp.dot(a, b, preferred_element_type=jnp.float32)


def _kernel(q_ref, k_ref, v_ref, sh_ref, kt_ref, dd_ref, w1_ref, w2_ref, w3_ref, w4_ref,
            f1_ref, mf_ref, mi_ref, g_ref, o_ref,
            kpad, kv_s, ra, rb, bo, y_s, h_s, h1_s):
    bf = jnp.bfloat16
    f32 = jnp.float32
    kpad[0:8, :] = jnp.zeros((8, D), f32)
    kpad[8:, :] = k_ref[...].astype(f32)

    def p1(i, c):
        r = pl.multiple_of(i * TM, TM)
        w = kpad[pl.ds(r, TM + 8), :]
        acc = w[8:] * sh_ref[0:1, :]
        for u in range(1, KS):
            acc = acc + w[8 - u:8 - u + TM] * sh_ref[u:u + 1, :]
        kv_s[pl.ds(i * 4, 4)] = (acc * v_ref[pl.ds(r, TM), :].astype(f32)).reshape(4, 8, 8, D)
        return c
    lax.fori_loop(0, S // TM, p1, 0)

    f1 = f1_ref[...]

    def s1(bk, c):
        xa = kv_s[:, bk].reshape(256, D).astype(bf)
        xb = kt_ref[:, bk].reshape(256, D).astype(bf)
        a = _dot(f1, xa).reshape(2 * HP, 8, D)
        b = _dot(f1, xb).reshape(2 * HP, 8, D)
        ra[:, bk] = a[:HP]
        ra[:, bk + 8] = a[HP:]
        rb[:, bk] = b[:HP]
        rb[:, bk + 8] = b[HP:]
        return c
    lax.fori_loop(0, 8, s1, 0)

    def s2(q, c):
        xa = _dot(mf_ref[q], ra[q].reshape(128, D).astype(bf))
        xb = _dot(mf_ref[q], rb[q].reshape(128, D).astype(bf))
        ar, ai, br, bi = xa[:64], xa[64:], xb[:64], xb[64:]
        yy = jnp.concatenate([ar * br - ai * bi, ar * bi + ai * br], axis=0)
        bo[q] = _dot(mi_ref[q], yy.astype(bf)).reshape(16, 8, D)
        return c
    lax.fori_loop(0, NK2, s2, 0)
    bo[NK2:] = jnp.zeros((HP - NK2, 16, 8, D), f32)

    g = g_ref[...]

    def s3(bk, c):
        z = jnp.concatenate([bo[:, bk], bo[:, bk + 8]], axis=0).reshape(2 * HP * 8, D)
        y_s[:, bk] = _dot(g, z.astype(bf)).reshape(32, 8, D)
        return c
    lax.fori_loop(0, 8, s3, 0)

    h1_s[0:8, :] = jnp.zeros((8, D), f32)
    h1_s[S + 8:, :] = jnp.zeros((8, D), f32)

    def p3(i, c):
        r = pl.multiple_of(i * TM, TM)
        x = q_ref[pl.ds(r, TM), :].astype(f32)
        yy = (y_s[pl.ds(i * 4, 4)] + kv_s[pl.ds(i * 4, 4)] * dd_ref[...]).reshape(TM, D)
        h = x + _ln(x) * yy
        h_s[pl.ds(r, TM), :] = h
        t = _ln(_ln(h))
        h1_s[pl.ds(r + 8, TM), :] = jax.nn.gelu(_dot(t.astype(bf), w1_ref[...]), approximate=True)
        return c
    lax.fori_loop(0, S // TM, p3, 0)

    col = lax.broadcasted_iota(jnp.int32, (TM, D), 1)
    c4 = D // 4

    def p4(i, c):
        r = pl.multiple_of(i * TM, TM)
        w = h1_s[pl.ds(r, TM + 16), :]
        hs_in = jnp.where(
            col < c4, w[7:7 + TM],
            jnp.where(col < 2 * c4, w[9:9 + TM],
                      jnp.where(col < 3 * c4, w[6:6 + TM], w[10:10 + TM])))
        h = h_s[pl.ds(r, TM), :]
        x1 = _ln(h) + _dot(hs_in.astype(bf), w2_ref[...])
        a = jax.nn.gelu(_dot(_ln(x1).astype(bf), w3_ref[...]), approximate=True)
        h2 = _dot(a.astype(bf), w4_ref[...])
        o_ref[pl.ds(r, TM), :] = (h + x1 + h2).astype(o_ref.dtype)
        return c
    lax.fori_loop(0, S // TM, p4, 0)


@jax.jit
def pallas_sequential_preLN__ssm_conv_h3__mixer_s_mlp__prompt_kernel(
    A_q, A_k, A_v, A_shift_k, A_ssm_k, A_ssm_D, B_x, B_w1, B_w2, B_w3, B_w4):
    f1, mf, mi, g = _consts()
    f32 = jnp.float32
    vm = lambda shape: pltpu.VMEM(shape, f32)
    out = pl.pallas_call(
        _kernel,
        out_shape=jax.ShapeDtypeStruct((S, D), A_q.dtype),
        scratch_shapes=[
            vm((S + 8, D)), vm((32, 8, 8, D)), vm((HP, 16, 8, D)), vm((HP, 16, 8, D)),
            vm((HP, 16, 8, D)), vm((32, 8, 8, D)), vm((S, D)), vm((S + 16, D)),
        ],
        compiler_params=pltpu.CompilerParams(vmem_limit_bytes=100 * 1024 * 1024),
    )(A_q.reshape(S, D), A_k.reshape(S, D), A_v.reshape(S, D),
      A_shift_k.T.astype(f32), A_ssm_k.T.astype(f32).reshape(32, 8, 8, D), A_ssm_D.reshape(1, D).astype(f32),
      B_w1, B_w2, B_w3, B_w4, f1, mf, mi, g)
    return out.reshape(1, S, D)
```
